```python
import jax
import jax.numpy as jnp

def _softmax(x, axis=-1):
    return jax.nn.softmax(x, axis=axis)
def _gelu(x):
    return jax.nn.gelu(x, approximate=True)
def _silu(x):
    return jax.nn.silu(x)
def _sigmoid(x):
    return jax.nn.sigmoid(x)
def _layernorm(x, axis=-1, eps=1e-5):
    m = jnp.mean(x, axis=axis, keepdims=True)
    v = jnp.var(x, axis=axis, keepdims=True)
    return (x - m) / jnp.sqrt(v + eps)
def _scatter_add(tgt, idx, src, axis=0):
    return tgt.at[idx].add(src)
def _segment_sum(src, seg, n):
    return jax.ops.segment_sum(src, seg, n)
class _Rng:
    def __init__(self, key):
        self._k = key
    def _next(self):
        self._k, sub = jax.random.split(self._k)
        return sub
    def normal(self, shape):
        return jax.random.normal(self._next(), shape, dtype=jnp.bfloat16)
    def randint(self, lo, hi, shape):
        return jax.random.randint(self._next(), shape, lo, hi, dtype=jnp.int32)
    def uniform(self, shape, lo=0.0, hi=1.0):
        return jax.random.uniform(self._next(), shape, jnp.bfloat16, lo, hi)
    def permutation(self, n):
        return jax.random.permutation(self._next(), n)


kernel_name = 'standalone__seq2seq_rnn_t_joint__speech'

def _fwd_setup_inputs():
    _rng = _Rng(jax.random.key(int.from_bytes(__import__("os").urandom(4), "little")))
    _w = (lambda a: (lambda t: t.astype(jnp.bfloat16) if jnp.issubdtype(t.dtype, jnp.floating) else t)(jnp.asarray(a)))
    B, T, D, K = 2, 1000, 512, 5
    U = 8
    sc = (1.0 / (K * D)) ** 0.5
    sd = (1.0 / D) ** 0.5
    return {
        "x": _w((lambda *s: _rng.normal(s) * 0.05)(B, T, D) * 0.5),
        "w1": _w((lambda *s: _rng.normal(s) * 0.05)(K, D, D) * sc),
        "w2": _w((lambda *s: _rng.normal(s) * 0.05)(K, D, D) * sc),
        "g": _w((lambda *s: _rng.normal(s) * 0.05)(B, U, D) * 0.5),
        "w_f": _w((lambda *s: _rng.normal(s) * 0.05)(D, D) * sd),
        "w_g": _w((lambda *s: _rng.normal(s) * 0.05)(D, D) * sd),
        "w_o": _w((lambda *s: _rng.normal(s) * 0.05)(D, D) * sd),
    }

def _fwd_reference(x, w1, w2, g, w_f, w_g, w_o):
    B, T, D = x.shape
    K = w1.shape[0]
    pad = K // 2
    xp = jnp.pad(x, ((0,0),(pad,pad),(0,0)))
    h = jnp.zeros_like(x)
    for i in range(K):
        h = h + jnp.einsum("btc,cd->btd", xp[:, i:i+T, :], w1[i])
    h = _gelu(h)[:, ::2, :]
    T1 = h.shape[1]
    hp = jnp.pad(h, ((0,0),(pad,pad),(0,0)))
    f = jnp.zeros_like(h)
    for i in range(K):
        f = f + jnp.einsum("btc,cd->btd", hp[:, i:i+T1, :], w2[i])
    f = _gelu(f)[:, ::2, :]
    fe = jnp.einsum("btd,de->bte", f, w_f)
    ge = jnp.einsum("bud,de->bue", g, w_g)
    j = jnp.tanh(fe[:, :, None, :] + ge[:, None, :, :])
    return jnp.einsum("btud,dv->btuv", j, w_o)


def setup_inputs():
    _inp = _fwd_setup_inputs()
    _gk = jax.random.fold_in(jax.random.key(int.from_bytes(__import__("os").urandom(4), "little")), 2**31 - 1)
    _shapes = [[2, 250, 8, 512]]
    _dtypes = ['bfloat16']
    _gks = jax.random.split(_gk, len(_shapes))
    _gs = [jax.random.normal(k, s, dtype=jnp.dtype(d)) * 0.05 for k, s, d in zip(_gks, _shapes, _dtypes)]
    _inp["grad_out"] = _gs[0]
    return _inp

def reference(x, w1, w2, g, w_f, w_g, w_o, grad_out):
    _const = dict()
    def _f(*_d):
        return _fwd_reference(**{'x': _d[0], 'w1': _d[1], 'w2': _d[2], 'g': _d[3], 'w_f': _d[4], 'w_g': _d[5], 'w_o': _d[6], **_const})
    _out, _vjp = jax.vjp(_f, x, w1, w2, g, w_f, w_g, w_o)
    _grads = _vjp(grad_out)
    _out0 = jnp.asarray(_out)
    return (_out0, *[jnp.asarray(_g) for _g in _grads])
```

```python
import jax
import jax.numpy as jnp
import jax.experimental.pallas as pl
import jax.experimental.pallas.tpu as pltpu

F32 = jnp.float32
BF16 = jnp.bfloat16
U32 = jnp.uint32

PA = 0.7
PB = 1.0 / PA
A2, B2 = PA * PA, PB * PB
S2 = A2 + B2
NA = PA / (2.0 * A2 * (A2 - B2))
NB = PB / (2.0 * B2 * (B2 - A2))

GC = 0.7978845608028654
GK = 0.044715

LANES = 128
JT = 32


def _nn(a, b):
    return jax.lax.dot_general(a, b, (((1,), (0,)), ((), ())), preferred_element_type=F32)


def _nt(a, b):
    return jax.lax.dot_general(a, b, (((1,), (1,)), ((), ())), preferred_element_type=F32)


def _tn(a, b):
    return jax.lax.dot_general(a, b, (((0,), (0,)), ((), ())), preferred_element_type=F32)


def _gelu_cdf(z):
    return 0.5 + 0.5 * jnp.tanh(z * (GC + (GC * GK) * (z * z)))


def _gelu_grad(z, cdf):
    return cdf + ((z * cdf) * (1.0 - cdf)) * (2.0 * GC + (6.0 * GC * GK) * (z * z))


def _data_fwd4(d):
    a2 = A2 * d[2]
    ea, oa = d[4] - B2 * d[2], PA * d[3] - PB * d[1]
    eb, ob = d[4] - a2, PB * d[3] - PA * d[1]
    v = [d[0] - a2 + ea, ea + oa, ea - oa, eb + ob, eb - ob]
    if len(d) == 6:
        v.append(d[1] - S2 * d[3] + d[5])
    return v


def _data_bwd4(v):
    sa, da, sb, db = v[1] + v[2], v[1] - v[2], v[3] + v[4], v[3] - v[4]
    sa, sb0 = sa + v[0], sb + v[0]
    d1 = (-PB) * da - PA * db
    d2 = (-B2) * sa - A2 * sb0
    d3 = PA * da + PB * db
    d4 = sa + sb
    if len(v) == 6:
        return [v[0], d1 + v[5], d2, d3 - S2 * v[5], d4, v[5]]
    return [v[0], d1, d2, d3, d4]


def _filt_fwd4(g):
    ea, eb = PB * g[0], PA * g[0]
    if len(g) == 3:
        ea, eb = ea + PA * g[2], eb + PB * g[2]
    return [g[0], ea + g[1], ea - g[1], eb + g[1], eb - g[1], *g[2:]]


def _filt_bwd4(u):
    sa, sb = u[1] + u[2], u[3] + u[4]
    g = [u[0] + PB * sa + PA * sb, (u[1] - u[2]) + (u[3] - u[4])]
    if len(u) == 6:
        g.append(u[5] + PA * sa + PB * sb)
    return g


def _out_fwd4(m):
    sa, da, sb, db = NA * (m[1] + m[2]), m[1] - m[2], NB * (m[3] + m[4]), m[3] - m[4]
    return [m[0] + sa + sb, (NA * PA) * da + (NB * PB) * db, A2 * sa + B2 * sb,
            (NA * A2 * PA) * da + (NB * B2 * PB) * db + m[5]]


def _out_bwd4(y):
    ea, oa = NA * (y[0] + A2 * y[2]), (NA * PA) * y[1] + (NA * A2 * PA) * y[3]
    eb, ob = NB * (y[0] + B2 * y[2]), (NB * PB) * y[1] + (NB * B2 * PB) * y[3]
    return [y[0], ea + oa, ea - oa, eb + ob, eb - ob, y[3]]


def _pack(lo, hi):
    return pltpu.pack_elementwise([lo, hi], packed_dtype=BF16)


def _unpack(words, odd):
    return pltpu.bitcast(words & U32(0xFFFF0000) if odd else words << 16, F32)


def _fold(parts):
    sub = jax.lax.broadcasted_iota(jnp.int32, parts[0].shape, 0)

    def merge(a, b, sh):
        return jnp.where((sub & sh) == 0, a + pltpu.roll(a, 8 - sh, 0), b + pltpu.roll(b, sh, 0))

    a, b = [merge(merge(q[0], q[2], 2), merge(q[1], q[3], 2), 1) for q in (parts[:4], parts[4:])]
    return jnp.where(sub < 4, a, pltpu.roll(b, 4, 0)), jnp.where(sub < 4, pltpu.roll(a, 4, 0), b)


def _sa(m):
    return [m[0] + m[3], m[2] + m[3], m[0], m[3], m[0] + m[1], m[2] - m[0], m[1] - m[3]]


def _sb(m):
    return [m[0] + m[3], m[0], m[1] - m[3], m[2] - m[0], m[3], m[0] + m[1], m[2] + m[3]]


def _sc(m):
    return [m[0] + m[3], m[2] - m[3], m[1] + m[3], m[0] + m[2], m[1] - m[0], m[3], m[0]]


def _sa_t(q):
    return [q[0] + q[4] + q[2] - q[5], q[4] + q[6], q[1] + q[5], q[0] + q[1] + q[3] - q[6]]


def _sb_t(q):
    return [q[0] + q[1] - q[3] + q[5], q[2] + q[5], q[3] + q[6], q[0] - q[2] + q[4] + q[6]]


def _sc_t(q):
    return [q[0] + q[3] - q[4] + q[6], q[2] + q[4], q[1] + q[3], q[2] - q[1] + q[0] + q[5]]


def _stage(steps):
    return lambda fn: lambda *args: (fn(*args), steps)


def _chain(*jobs):
    def run():
        for gen, _ in jobs:
            yield from gen

    return run(), sum(n for _, n in jobs)


def _weave(jobs, span):
    live = [[gen, n, 0, (0.0, 1.0) if i == 0 else span] for i, (gen, n) in enumerate(jobs)]
    while live:
        job = min(live, key=lambda e: e[3][0] + (e[3][1] - e[3][0]) * (e[2] + 0.5) / e[1])
        job[2] += 1
        if next(job[0], "done") == "done":
            live = [e for e in live if e is not job]


def _kernel(x_h, w1_h, w2_h, g_h, wf_h, wg_h, wo_h, go_h,
            out_h, dx_h, dw1_h, dw2_h, dg_h, dwf_h, dwg_h, dwo_h,
            x_v, w1_v, w2_v, g_v, wf_v, wg_v, wo_v, go_v,
            dg_v, dwg_v,
            xs, u1, v1, gp1, u2, v2, gp2, fa, fe_v, djq, ja, gc, wob, wfb, acc, dfe_v, dfc,
            dm2, dm1, ge_v, dge_v, oq, pa, pb, pc, pd, pe, pf, isem, osem, *, step, nb, per_b):
    out_v, dx_v, dw1_v, dw2_v, dwf_v, dwo_v = go_v, x_v, w1_v, w2_v, wf_v, wo_v
    nt = nb * per_b
    mp = gp1[0].shape[1]
    mh = mp // 2
    d = wo_v.shape[0]
    dh = d // 2
    nu = g_v.shape[0] // nb
    npair = dh // LANES
    chunks = [(t0, min(JT, nt - t0)) for t0 in range(0, nt, JT)]
    half = 8 * JT

    def col(c, base=0):
        return slice(base + c * LANES, base + (c + 1) * LANES)

    def pair(p):
        return slice(2 * p * LANES, (2 * p + 2) * LANES)

    def rows(t0, n):
        return pl.ds(16 * t0, 16 * n)

    def save(ref, idx, r0, where, lo, hi):
        ref[(*idx, pl.ds(r0 // 2, lo.shape[0]), where)] = _pack(lo, hi)

    def get(ref, i, *idx):
        return ref[(i, *idx)]

    def load(ref, idx, r0, n, where):
        return pltpu.bitcast(get(ref, *idx, pl.ds(r0 // 2, n // 2), where), BF16)

    def spread(ref, idx, r0, where, comb, lo, hi):
        for r, (a, b) in enumerate(zip(comb(lo), comb(hi))):
            save(ref, (*idx, r), r0, where, a, b)

    def wwords(ref, idx, p, s, i0):
        return [pltpu.bitcast(ref[(*idx, pl.ds((2 * p + i) * LANES + i0, 16), col(2 * s + k))], U32)
                for i in range(2) for k in range(2)]

    def wquads(ref, idx, p, s, i0):
        w = wwords(ref, idx, p, s, i0)
        return [[_unpack(a, odd) for a in w] for odd in range(2)]

    def piece(i0):
        return pl.ds(i0 // 16 * 16 + i0 // 8 % 2, 8, stride=2)

    sources = {"wo": (wo_h, wo_v), "wf": (wf_h, wf_v), "wg": (wg_h, wg_v), "g": (g_h, g_v)}
    for c, ch in enumerate(chunks):
        sources["go", c] = (go_h.at[rows(*ch)], go_v.at[rows(*ch)])
    for p in range(npair):
        for c in (2 * p, 2 * p + 1):
            sources["x", c] = (x_h.at[:, col(c)], x_v.at[:, col(c)])
        for s in range(npair):
            sources["w1", p, s] = (w1_h.at[:, pair(p), pair(s)], w1_v.at[:, pair(p), pair(s)])
            sources["w2", p, s] = (w2_h.at[:, pair(p), pair(s)], w2_v.at[:, pair(p), pair(s)])
    loads = {name: pltpu.make_async_copy(src, dst, isem.at[i])
             for i, (name, (src, dst)) in enumerate(sources.items())}

    def fetch(*names):
        for name in names:
            loads[name].start()

    def arrive(*names):
        for name in names:
            loads[name].wait()

    stores = []

    def put(src, dst):
        cp = pltpu.make_async_copy(src, dst, osem.at[len(stores)])
        cp.start()
        stores.append(cp)

    sub = jax.lax.broadcasted_iota(jnp.int32, (8, LANES), 0)
    firsts = [b * per_b for b in range(nb + 1)]
    lasts = [b * per_b - 1 for b in range(1, nb + 1)]

    def drop(a, t0, tiles):
        for t in tiles:
            if t0 <= t < t0 + 8:
                a = jnp.where(sub == t - t0, jnp.zeros_like(a), a)
        return a

    def from_prev(get, t0):
        a = get(t0) if t0 == 0 else jnp.where(sub == 7, get(t0 - 8), get(t0))
        return drop(pltpu.roll(a, 1, 0), t0, firsts)

    def from_next(get, t0):
        a = get(t0) if t0 + 8 == mp else jnp.where(sub == 0, get(t0 + 8), get(t0))
        return drop(pltpu.roll(a, 7, 0), t0, lasts + [mp - 1])

    def sweep(produce, finish):
        for i0 in range(0, mh, 8):
            yield from produce(i0)
            if i0 % 16 == 0 and i0 >= 32:
                yield from finish(i0 - 16)
        yield from finish(mh - 16)
        yield from finish(0)

    every = slice(None)

    @_stage(32)
    def plain_weight(src, dst, ps):
        for p in ps:
            for s in range(npair):
                for i0 in range(0, LANES, 16):
                    spread(dst, (), p * LANES + i0, col(s), _sb, *wquads(src, (), p, s, i0))
                    yield

    @_stage(32)
    def go_prep(c):
        t0, n = chunks[c]
        for i in range(n // 2):
            for p in range(npair):
                w = [pltpu.bitcast(go_v[rows(t, 1), col(2 * p + k)], U32)
                     for t in (t0 + i, t0 + n // 2 + i) for k in range(2)]
                lo, hi = [_sc([_unpack(a, odd) for a in w])[:5] for odd in range(2)]
                for r, a in enumerate([_pack(*e) for e in zip(lo, hi)] + [w[3], w[0]]):
                    gc[c][r, pl.ds(8 * i, 8), col(p)] = a
                yield
        if n < JT:
            for ref in (gc[c], ja[c]):
                ref[:, 4 * n:, :] = jnp.zeros((7, half // 2 - 4 * n, dh), U32)

    def by_pair(dst, r, where, val):
        for s in range(npair):
            dst[r, s, where, :] = val[:, col(s)]

    @_stage(14)
    def dj_mm(c):
        n = 8 * chunks[c][1]
        for r in range(7):
            for s in range(npair):
                djq[c][r, s, 0:n, :] = _nt(load(gc[c], (r,), 0, n, every), load(wob, (r,), s * LANES, LANES, every))
                yield

    @_stage(88)
    def x_prep(p):
        for c in range(2):
            xs[p][c, 0:8, :] = jnp.zeros((8, LANES), U32)
            xs[p][c, 8 + 4 * nt:, :] = jnp.zeros((4 * (mp - nt) + 8, LANES), U32)
            for t in range(0, nt, 64):
                n = min(64, nt - t)
                xs[p][c, pl.ds(8 + 4 * t, 4 * n), :] = pltpu.bitcast(
                    x_v[pl.ds(8 * t, 8 * n), col(2 * p + c)], U32)
                yield
        for i0 in range(0, mh, 16):
            for odd in range(2):
                q = [[], []]
                for e in range(2):
                    for t0 in (i0 + 8 * e, mh + i0 + 8 * e):
                        for c in range(2):
                            w = [xs[p][c, pl.ds(7 + k + 4 * t0, 8, stride=4), :] for k in range(6 - odd)]
                            w[0] = drop(w[0], t0, firsts)
                            if not odd:
                                w[5] = drop(w[5], t0, lasts)
                            q[e].append(_data_fwd4([_unpack(a, odd) for a in w]))
                        yield
                for k in range(6 - odd):
                    spread(v1[p], (k,), i0, col(odd), _sa, *[[a[k] for a in e] for e in q])
                yield

    @_stage(32)
    def w1_prep(p, s):
        for i0 in range(0, LANES, 16):
            for odd in range(2):
                g = [wquads(w1_v, (i,), p, s, i0) for i in range(odd, 5, 2)]
                f = [[_filt_fwd4([a[e][n] for a in g]) for n in range(4)] for e in range(2)]
                yield
                for k in range(6 - odd):
                    spread(u1[p][s], (k,), odd * LANES + i0, every, _sb, *[[a[k] for a in e] for e in f])
                yield

    @_stage(32)
    def w2_prep(p, s):
        def points(g):
            if len(g) == 2:
                return g[0], g[0] + g[1], g[1]
            e = g[0] + g[2]
            return g[0], e + g[1], g[2], e - g[1]

        for i0 in range(0, LANES, 16):
            for odd in range(2):
                g = [wquads(w2_v, (i,), p, s, i0) for i in range(odd, 5, 2)]
                f = [[points([a[e][n] for a in g]) for n in range(4)] for e in range(2)]
                yield
                for k in range(4 - odd):
                    spread(u2[p][s], (k,), odd * LANES + i0, every, _sb, *[[a[k] for a in e] for e in f])
                yield

    def flip_steps(ref):
        n = ref.shape[0]
        for k in range(n):
            for r in range(7):
                for odd in range(2 if k < n - 1 else 1):
                    ref[k, r, :, col(odd)] = pltpu.bitcast(load(ref, (k, r), 0, mh, col(odd)).T, U32)
                yield

    @_stage(7)
    def flip_j(c):
        for r in range(7):
            ja[c][r] = pltpu.bitcast(load(ja[c], (r,), 0, half, every).T, U32)
            yield

    def fwd_mm_steps(v, u, ps, s, res):
        n = v[0].shape[0]
        for k in range(n):
            kd = LANES * (2 if k < n - 1 else 1)
            for r in range(7):
                m = res[k, r] if ps[0] else None
                for p in ps:
                    part = _nn(load(v[p], (k, r), 0, mh, slice(0, kd)), load(u[p][s], (k, r), 0, kd, every))
                    m = part if m is None else m + part
                    if p != ps[-1]:
                        yield
                res[k, r] = m
                yield

    def dx_mm_steps(dm, u, p, res):
        n = dm[0].shape[0]
        for k in range(n):
            nd = 2 if k < n - 1 else 1
            for r in range(7):
                m = _nt(jnp.concatenate([load(a, (k, r), 0, mh, every) for a in dm], axis=1),
                        jnp.concatenate([load(a, (k, r), 0, nd * LANES, every) for a in u[p]], axis=1))
                for odd in range(nd):
                    res[odd * n + k, r] = m[:, col(odd)]
                yield

    def dw_mm_steps(v, dm, p, res):
        n = dm[0].shape[0]
        for k in range(n):
            nd = 2 if k < n - 1 else 1
            for r in range(7):
                a = jnp.concatenate([load(v[p], (k, r), 0, mh, col(odd)) for odd in range(nd)], axis=0)
                for s in range(npair):
                    m = _nn(a, load(dm[s], (k, r), 0, mh, every))
                    for odd in range(nd):
                        res[odd][s * n + k, r] = m[col(odd)]
                yield

    steps = (flip_steps, fwd_mm_steps, dx_mm_steps, dw_mm_steps)
    flip1, fwd1_mm, dx1_mm, dw1_mm = map(_stage(42), steps)
    flip2, fwd2_mm, dx2_mm, dw2_mm = map(_stage(28), steps)

    def gather(res, k, where, comb):
        return comb([get(res, k, r, where) for r in range(7)])

    @_stage(136)
    def conv1_post(s, res):
        h = {}

        def produce(i0):
            m = [gather(res, k, piece(i0), _sc_t) for k in range(6)]
            yield
            for n in range(4):
                t0, c = (n // 2) * mh + i0, 2 * s + n % 2
                for q, z in enumerate(_out_fwd4([a[n] for a in m])):
                    cdf = _gelu_cdf(z)
                    h[q, c, t0] = z * cdf
                    gp1[s][q, pl.ds(t0, 8), col(n % 2)] = z
                    gp1[s][4 + q, pl.ds(t0, 8), col(n % 2)] = cdf
                yield

        def point(k, c, t):
            if k == 0:
                return from_prev(lambda e: h[2, c, e], t) - h[2, c, t]
            if k == 2:
                return from_next(lambda e: h[0, c, e], t) - h[0, c, t]
            if k == 4:
                return from_prev(lambda e: h[3, c, e], t) - h[1, c, t]
            if k == 1:
                return 0.5 * (h[0, c, t] + h[2, c, t])
            if k == 3:
                return 0.5 * (h[2, c, t] - h[0, c, t])
            return h[1, c, t] if k == 5 else h[3, c, t] - h[1, c, t]

        def finish(i0):
            for k in range(7):
                q = [[point(k, c, t + e) for t in (i0, mh + i0) for c in (2 * s, 2 * s + 1)] for e in (0, 8)]
                spread(v2[s], (k % 4,), i0, col(k // 4), _sa, *q)
                yield

        return sweep(produce, finish)

    @_stage(96)
    def conv2_post(s, res):
        for i0 in range(0, mh, 16):
            y = {}
            for i in (i0, i0 + 8):
                m = [gather(res, k, piece(i), _sc_t) for k in range(4)]
                yield
                for n in range(4):
                    for r, z in enumerate((m[0][n] + m[1][n] + m[3][n], m[1][n] - m[3][n] + m[2][n])):
                        where = (pl.ds((n // 2) * mh + i, 8), col(2 * s + n % 2))
                        cdf = _gelu_cdf(z)
                        y[r, n, i] = z * cdf
                        gp2[(r, *where)] = z
                        gp2[(2 + r, *where)] = cdf
                    yield
            for r in range(2):
                spread(fa[s], (), r * mh + i0, every, _sa, *[[y[r, n, i] for n in range(4)] for i in (i0, i0 + 8)])
                yield

    @_stage(64)
    def gelu_grad(ref):
        n = ref.shape[0] // 2
        for q in range(n):
            for t0 in range(0, mp, 4 * n):
                ref[q, pl.ds(t0, 4 * n), :] = _gelu_grad(ref[q, pl.ds(t0, 4 * n), :], ref[n + q, pl.ds(t0, 4 * n), :])
                yield

    @_stage(1)
    def ge_mm():
        m = _nn(g_v[...], wg_v[...])
        for k in range(2 * npair):
            ge_v[k] = m[:, col(k)]
        dge_v[...] = jnp.zeros(dge_v.shape, F32)
        yield

    @_stage(7)
    def fe_mm(p):
        for r in range(7):
            m = _nn(load(fa[p], (r,), 0, mp, every), load(wfb, (r,), p * LANES, LANES, every))
            for s in range(npair):
                oq[1][r, s] = m[:, col(s)] if p == 0 else get(oq[1], r, s) + m[:, col(s)]
            yield

    @_stage(16)
    def fe_post(lo, hi):
        for i0 in range(lo, hi, 8):
            for r in range(2):
                for s in range(npair):
                    q = _sc_t([oq[1][k, s, piece(r * mh + i0), :] for k in range(7)])
                    for n in range(4):
                        fe_v[r, pl.ds((n // 2) * mh + i0, 8), col(2 * s + n % 2)] = q[n]
                yield

    @_stage(288)
    def joint_act(c):
        t0, n = chunks[c]
        seqs = sorted({t // per_b for t in range(t0, t0 + n)})
        for p in range(npair):
            done, ge, dge = {}, {}, {}
            ks = (2 * p, 2 * p + 1)
            for key in [(b, k, e) for b in seqs for k in ks for e in range(2)]:
                b, k, e = key
                a = ge_v[k, pl.ds(e, 8, stride=2), :]
                ge[key] = jnp.where((sub < 4) == (b == 0), a, pltpu.roll(a, 4, 0))
                dge[key] = dge_v[b, e, :, col(k)]
            for i in range(n // 2):
                ts = (t0 + i, t0 + n // 2 + i)
                dj = [_sa_t([djq[c][r, p, pl.ds(16 * i + e, 8, stride=2), :] for r in range(7)])
                      for e in range(2)]
                jq = [[], []]
                yield
                for m in range(4):
                    t, k = ts[m // 2], 2 * p + m % 2
                    b = t // per_b
                    fe = jnp.where(sub < 4, *[
                        jnp.broadcast_to(get(fe_v, r, pl.ds(t, 1), col(k)), (nu, LANES)) for r in range(2)])
                    z = []
                    for e in range(2):
                        j = jnp.tanh(fe + ge[b, k, e])
                        z.append(dj[e][m] * (1.0 - j * j))
                        dge[b, k, e] = dge[b, k, e] + z[e]
                        jq[e].append(j)
                        if e == 0:
                            yield
                    done[t, k] = z[0] + z[1]
                    yield
                spread(ja[c], (), 16 * i, col(p), _sa, *jq)
                for s0 in range(t0, t0 + JT, 8):
                    group = range(s0, min(s0 + 8, nt))
                    if s0 not in done and all((t, 2 * p) in done for t in group):
                        done[s0] = None
                        for k in ks:
                            part = [done[t, k] for t in group]
                            part += [jnp.zeros((nu, LANES), F32)] * (8 - len(part))
                            for r, a in enumerate(_fold(part)):
                                dfe_v[r, pl.ds(s0, 8), col(k)] = a
                if i + 1 == n // 2:
                    for (b, k, e), a in dge.items():
                        dge_v[b, e, :, col(k)] = a

    @_stage(14)
    def out_mm(c):
        n = 8 * chunks[c][1]
        for r in range(7):
            for s in range(npair):
                djq[c][r, s, 0:n, :] = _nn(load(ja[c], (r,), 0, n, every), load(wob, (r,), 0, dh, col(s)))
                yield

    @_stage(32)
    def out_post(c):
        t0, n = chunks[c]
        for i in range(n // 2):
            for p in range(npair):
                q = _sc_t([get(djq[c], r, p, pl.ds(16 * i, 16)) for r in range(7)])
                for m in range(4):
                    out_v[rows(t0 + (m // 2) * (n // 2) + i, 1), col(2 * p + m % 2)] = q[m].astype(BF16)
                yield

    def dwo_mm(c, prev, res):
        return dwo_steps((c,), prev, res), 14

    def dwo_steps(cs, prev, res):
        for r in range(7):
            m = None if prev is None else jnp.concatenate([prev[r, s] for s in range(npair)], axis=1)
            for c in cs:
                q = []
                for s in range(npair):
                    q.append(_tn(load(ja[c], (r,), 0, half, col(s)), load(gc[c], (r,), 0, half, every)))
                    if s == 0:
                        yield
                q = jnp.concatenate(q, axis=0)
                m = q if m is None else m + q
                yield
            by_pair(res, r, every, m)

    @_stage(28)
    def dwo_rest(cs, p, prev, res):
        for r in range(7):
            m = jnp.concatenate([prev[r, s, col(p), :] for s in range(npair)], axis=1)
            for c in cs:
                m = m + _nn(load(ja[c], (r,), p * LANES, LANES, every), load(gc[c], (r,), 0, half, every))
                yield
            by_pair(res, r, col(p), m)

    def store_weight(dst, idx, p, s, i0, q):
        for n in range(4):
            dst[(*idx, pl.ds((2 * p + n // 2) * LANES + i0, q[n].shape[0]), col(2 * s + n % 2))] = (
                q[n].astype(BF16))

    @_stage(16)
    def plain_dw_post(src, dst, ps=(0, 1)):
        for p in ps:
            for i0 in range(0, LANES, 16):
                for s in range(npair):
                    store_weight(dst, (), p, s, i0,
                                 _sb_t([get(src, r, s, pl.ds(p * LANES + i0, 16)) for r in range(7)]))
                    yield

    @_stage(32)
    def df_prep():
        for r in range(2):
            for i0 in range(0, mh, 16):
                for s in range(npair):
                    q = [[get(dfe_v, r, pl.ds((n // 2) * mh + i, 8), col(2 * s + n % 2)) for n in range(4)]
                         for i in (i0, i0 + 8)]
                    spread(dfc, (), r * mh + i0, col(s), _sc, *q)
                    yield

    @_stage(14)
    def df_mm():
        for r in range(7):
            for s in range(npair):
                oq[0][r, s] = _nt(load(dfc, (r,), 0, mp, every), load(wfb, (r,), s * LANES, LANES, every))
                yield

    @_stage(48)
    def df_post():
        for i0 in range(0, mh, 16):
            for s in range(npair):
                y = {}
                for i in (i0, i0 + 8):
                    for r in range(2):
                        q = _sa_t([oq[0][k, s, piece(r * mh + i), :] for k in range(7)])
                        y[i, r] = _sc([q[n] * gp2[r, pl.ds((n // 2) * mh + i, 8), col(2 * s + n % 2)]
                                       for n in range(4)])
                    yield
                for r in range(7):
                    m = [(a, a + b, b, a - b) for a, b in [(y[i, 0][r], y[i, 1][r]) for i in (i0, i0 + 8)]]
                    for k in range(4):
                        save(dm2[s], (k, r), i0, every, m[0][k], m[1][k])
                yield

    @_stage(14)
    def dwf_mm():
        for r in range(7):
            for p in range(npair):
                by_pair(oq[1], r, col(p), _tn(load(fa[p], (r,), 0, mp, every), load(dfc, (r,), 0, mp, every)))
                yield

    @_stage(2)
    def dg_mm():
        low = jax.lax.broadcasted_iota(jnp.int32, (8, d), 0) < 4
        m = [jnp.where(low, *[dge_v[b, e] + pltpu.roll(dge_v[b, e], 4, 0) for b in range(nb)])
             for e in range(2)]
        dge = pltpu.bitcast(_pack(*m), BF16)
        dg_v[...] = _nt(dge, wg_v[...]).astype(BF16)
        yield
        dwg_v[...] = _tn(g_v[...], dge).astype(BF16)
        yield

    @_stage(96)
    def conv2_dx_post(p, res):
        w = {}

        def produce(i0):
            e = [gather(res, k, piece(i0), _sa_t) for k in range(4)]
            for n in range(4):
                key = (2 * p + n % 2, (n // 2) * mh + i0)
                e0, e1, e2, e3 = [a[n] for a in e]
                w[(0, *key)], w[(2, *key)] = 0.5 * (e1 - e3) - e2, 0.5 * (e1 + e3) - e0
                w[(4, *key)], w[(5, *key)] = e2, e0
            yield
            o = [gather(res, 4 + k, piece(i0), _sa_t) for k in range(3)]
            for n in range(4):
                key = (2 * p + n % 2, (n // 2) * mh + i0)
                w[(1, *key)], w[(3, *key)], w[(6, *key)] = o[1][n] - o[0][n] - o[2][n], o[2][n], o[0][n]
            yield

        def dz(q, c, t):
            a = w[q, c, t]
            if q == 0:
                a = a + from_prev(lambda e: w[4, c, e], t)
            elif q >= 2:
                a = a + from_next(lambda e: w[q + 3, c, e], t)
            return a * gp1[p][q, pl.ds(t, 8), col(c % 2)]

        def finish(i0):
            y = [[_sc([dz(q, c, t + e) for t in (i0, mh + i0) for c in (2 * p, 2 * p + 1)])
                  for q in range(4)] for e in (0, 8)]
            yield
            for r in range(7):
                for k, a in enumerate(zip(*[_out_bwd4([a[r] for a in e]) for e in y])):
                    save(dm1[p], (k, r), i0, every, *a)
                yield

        return sweep(produce, finish)

    @_stage(64)
    def conv2_dw_post(p, odd, res):
        for i0 in range(0, LANES, 8):
            for s in range(npair):
                m = [gather(res, 4 * s + k, pl.ds(i0, 8), _sb_t) for k in range(4 - odd)]
                if odd:
                    g = {1: [a + b for a, b in zip(m[0], m[1])], 3: [a + b for a, b in zip(m[1], m[2])]}
                else:
                    e = [a + b for a, b in zip(m[1], m[3])]
                    g = {0: [a + b for a, b in zip(m[0], e)], 4: [a + b for a, b in zip(m[2], e)],
                         2: [a - b for a, b in zip(m[1], m[3])]}
                yield
                for i, q in g.items():
                    store_weight(dw2_v, (i,), p, s, i0, q)
                yield

    @_stage(104)
    def conv1_dx_post(p, res):
        w = {}

        def emit(k, c, t, ev, od):
            xs[p][c, pl.ds(k + 4 * t, 8, stride=4), :] = _pack(ev, od)

        def points(ks, t):
            q = [[res[k, r, piece(t % mh), :] for r in range(7)] for k in ks]
            if t < mh:
                return [a[0] + a[4] + a[2] - a[5] for a in q], [a[4] + a[6] for a in q]
            return [a[1] + a[5] for a in q], [a[0] + a[1] + a[3] - a[6] for a in q]

        def end(c, t):
            emit(3, c, t, *[w[c, t][k][4] + from_next(lambda e: w[c, e][k][0], t) for k in range(2)])

        for t in range(0, mp, 8):
            ev = [_data_bwd4(a) for a in points(range(6), t)]
            yield
            for c, a, b in zip(range(2), ev, points(range(6, 11), t)):
                b = _data_bwd4(b)
                w[c, t] = (a, b)
                emit(0, c, t, a[1] + from_prev(lambda e: w[c, e][0][5], t), b[1])
                emit(1, c, t, a[2], b[2])
                emit(2, c, t, a[3], b[3])
                if t:
                    end(c, t - 8)
                yield
        for c in range(2):
            end(c, mp - 8)
            for t in range(0, nt, 32):
                n = min(32, nt - t)
                dx_v[pl.ds(8 * t, 8 * n), col(2 * p + c)] = pltpu.bitcast(xs[p][c, pl.ds(4 * t, 4 * n), :], BF16)
                if t % 64:
                    yield

    @_stage(64)
    def conv1_dw_post(p, odd, res):
        for i0 in range(0, LANES, 8):
            for s in range(npair):
                m = [gather(res, 6 * s + k, pl.ds(i0, 8), _sb_t) for k in range(6 - odd)]
                yield
                g = [_filt_bwd4([a[n] for a in m]) for n in range(4)]
                for k, i in enumerate(range(odd, 5, 2)):
                    store_weight(dw1_v, (i,), p, s, i0, [a[k] for a in g])
                yield

    nc = len(chunks)
    assert nc == 8 and npair == 2

    blocks = []

    def block(*jobs, need=(), span=(0.0, 1.0)):
        arrive(*need)
        blocks.append(jobs)
        pl.when(step < len(blocks))(lambda: _weave(jobs, span))

    def split(job, n):
        gen, total = job
        return ((next(gen) for _ in range(n)), n), (gen, total - n)

    def dj_whole(c):
        def run():
            for _ in go_prep(c)[0]:
                pass
            yield from dj_mm(c)[0]

        return run(), dj_mm(c)[1]

    def go(*cs):
        return [("go", c) for c in cs]

    def put_out(c):
        put(out_v.at[rows(*chunks[c])], out_h.at[rows(*chunks[c])])

    def put_dw1(p, taps):
        for i in taps:
            put(dw1_v.at[i, pair(p), :], dw1_h.at[i, pair(p), :])

    fetch("wo", *go(0, 1, 2, 3), *go(4), ("x", 0), ("x", 1), *go(5, 6), ("w1", 0, 0),
          ("x", 2), ("x", 3), ("w1", 1, 0), ("w1", 0, 1), ("w1", 1, 1), ("w2", 0, 0), ("w2", 0, 1), ("w2", 1, 0),
          ("w2", 1, 1), "wf", *go(7), "g", "wg")
    x0, x1 = split(x_prep(0), 38), split(x_prep(1), 48)
    block(plain_weight(wo_v, wob, (0, 1)), need=["wo"])
    block(dj_whole(0), need=go(0))
    block(dj_whole(1), need=go(1))
    block(_chain(dj_whole(2), dj_whole(3)), need=go(2, 3))
    block(dj_whole(4), x0[0], need=[*go(4), ("x", 0), ("x", 1)])
    block(dj_whole(5), x0[1], need=go(5))
    block(dj_whole(6), w1_prep(0, 0), need=[*go(6), ("w1", 0, 0)])
    block(fwd1_mm(v1, u1, (0,), 0, pa), _chain(*x1), w1_prep(1, 0), need=[("x", 2), ("x", 3), ("w1", 1, 0)])
    block(fwd1_mm(v1, u1, (1,), 0, pa), _chain(w1_prep(0, 1), w1_prep(1, 1)), need=[("w1", 0, 1), ("w1", 1, 1)])
    block((fwd1_mm(v1, u1, (0, 1), 1, pb)[0], 84), conv1_post(0, pa), _chain(w2_prep(0, 0), w2_prep(0, 1), w2_prep(1, 0)),
          need=[("w2", 0, 0), ("w2", 0, 1), ("w2", 1, 0)])
    block(_chain(fwd2_mm(v2, u2, (0,), 0, pa), fwd2_mm(v2, u2, (0,), 1, pc)), conv1_post(1, pb))
    block(fwd2_mm(v2, u2, (1,), 0, pa), w2_prep(1, 1), plain_weight(wf_v, wfb, (0, 1)),
          need=[("w2", 1, 1), "wf"])
    block(fwd2_mm(v2, u2, (1,), 1, pc), conv2_post(0, pa), go_prep(7), need=go(7))
    block(_chain(fe_mm(0), ge_mm()), conv2_post(1, pc), need=["g", "wg"])
    g2 = split(gelu_grad(gp2), 40)
    block(fe_mm(1), g2[0])
    block(dj_mm(7), _chain(fe_post(0, mh // 2), joint_act(0)))
    block(_chain(out_mm(0), dwo_mm(0, None, acc[0])), _chain(joint_act(1), fe_post(mh // 2, mh), joint_act(2)))
    block(_chain(out_mm(1), out_mm(2), (dwo_steps((1, 2), acc[0], acc[1]), 28)),
          _chain(joint_act(3), joint_act(4)), out_post(0))
    put_out(0)
    block(_chain(out_mm(3), dwo_mm(3, acc[1], acc[0]), out_mm(4)), _chain(joint_act(5), joint_act(6)),
          _chain(out_post(1), out_post(2)))
    put_out(1)
    put_out(2)
    block(_chain(out_mm(5), out_mm(6)), joint_act(7), out_post(3), g2[1])
    put_out(3)
    block(out_mm(7), df_prep(), out_post(4))
    block(df_mm(), _chain(out_post(5), out_post(6)))
    put_out(4)
    put_out(5)
    block(_chain(dg_mm(), dwf_mm()), df_post())
    put_out(6)
    block(_chain(dx2_mm(dm2, u2, 0, pa), dx2_mm(dm2, u2, 1, pb)), _chain(flip2(v2[0]), flip2(v2[1])), out_post(7), gelu_grad(gp1[0]), gelu_grad(gp1[1]),
          plain_dw_post(oq[1], dwf_v, (0,)), plain_dw_post(oq[1], dwf_v, (1,)))
    put_out(7)
    for src, dst in ((dg_v, dg_h), (dwg_v, dwg_h), (dwf_v, dwf_h)):
        put(src, dst)
    block(dw2_mm(v2, dm2, 0, (pc, pd)), conv2_dx_post(0, pa))
    block(dw2_mm(v2, dm2, 1, (pa, pe)), conv2_dx_post(1, pb), flip1(v1[0]))
    block(dw1_mm(v1, dm1, 0, (pf, pb)), flip1(v1[1]),
          _chain(*[conv2_dw_post(i // 2, i % 2, a) for i, a in enumerate((pc, pd, pa, pe))]))
    put(dw2_v, dw2_h)
    block(dw1_mm(v1, dm1, 1, (pa, pe)),
          _chain(conv1_dw_post(0, 0, pf), conv1_dw_post(0, 1, pb)))
    put_dw1(0, range(5))
    block(dx1_mm(dm1, u1, 0, pc), _chain(*map(flip_j, (4, 5, 6, 7))),
          _chain(conv1_dw_post(1, 0, pa), conv1_dw_post(1, 1, pe)))
    put_dw1(1, range(5))
    block(dx1_mm(dm1, u1, 1, pd), conv1_dx_post(0, pc))
    put(dx_v.at[:, pair(0)], dx_h.at[:, pair(0)])
    block(dwo_rest((4, 5, 6, 7), 0, acc[0], acc[1]), conv1_dx_post(1, pd))
    put(dx_v.at[:, pair(1)], dx_h.at[:, pair(1)])
    block(dwo_rest((4, 5, 6, 7), 1, acc[0], oq[0]), plain_dw_post(acc[1], dwo_v, (0,)))
    put(dwo_v.at[pair(0)], dwo_h.at[pair(0)])
    block(plain_dw_post(oq[0], dwo_v, (1,)))
    put(dwo_v.at[pair(1)], dwo_h.at[pair(1)])
    for cp in stores:
        cp.wait()


@jax.jit
def pallas_standalone__seq2seq_rnn_t_joint__speech_kernel(
    x: jax.Array,
    w1: jax.Array,
    w2: jax.Array,
    g: jax.Array,
    w_f: jax.Array,
    w_g: jax.Array,
    w_o: jax.Array,
    grad_out: jax.Array,
):
    nb, t, d = x.shape
    nu = g.shape[1]
    assert w1.shape[0] == 5 and t % 8 == 0 and nb == 2 and nu == 8 and d % LANES == 0
    per_b = t // 8
    nt = nb * per_b
    mp = (nt // JT + 1) * JT

    args = [x.reshape(nb * t, d), w1, w2, g.reshape(nb * nu, d), w_f, w_g, w_o,
            grad_out.reshape(16 * nt, d)]
    args = [a.astype(BF16) for a in args]
    outs = [args[7]] + args[:7]
    vm = pltpu.VMEM
    scratch = (
        [vm(a.shape, BF16) for a in args]
        + [vm(args[3].shape, BF16), vm(args[5].shape, BF16)]
        + [
            [vm((2, 4 * mp + 16, LANES), U32)] * 2,
            [[vm((6, 7, LANES, LANES), U32)] * 2] * 2,
            [vm((6, 7, mp // 4, 2 * LANES), U32)] * 2,
            [vm((8, mp, 2 * LANES), F32)] * 2,
            [[vm((4, 7, LANES, LANES), U32)] * 2] * 2,
            [vm((4, 7, mp // 4, 2 * LANES), U32)] * 2,
            vm((4, mp, d), F32),
            [vm((7, mp // 2, LANES), U32)] * 2,
            vm((2, mp, d), F32),
            [vm((7, 2, 8 * JT, LANES), F32)] * (mp // JT),
            [vm((7, 4 * JT, d // 2), U32)] * (mp // JT),
            [vm((7, 4 * JT, d // 2), U32)] * (mp // JT),
            vm((7, d // 4, d // 2), U32),
            vm((7, d // 4, d // 2), U32),
            [vm((7, 2, d // 2, LANES), F32)] * 2,
            vm((2, mp, d), F32),
            vm((7, mp // 2, d // 2), U32),
            [vm((4, 7, mp // 4, LANES), U32)] * 2,
            [vm((6, 7, mp // 4, LANES), U32)] * 2,
            vm((d // LANES, nb * nu, LANES), F32),
            vm((nb, 2, nu, d), F32),
            [vm((7, 2, mp, LANES), F32)] * 2,
            *[vm((n, 7, LANES, LANES), F32) for n in (12, 11, 11, 11, 11, 12)],
            pltpu.SemaphoreType.DMA((32,)),
            pltpu.SemaphoreType.DMA((32,)),
        ]
    )

    def kernel(*refs):
        step = jax.lax.fori_loop(0, 2, lambda i, c: c * i, 1)
        with jax.disable_jit():
            _kernel(*refs, step=step, nb=nb, per_b=per_b)

    res = pl.pallas_call(
        kernel,
        in_specs=[pl.BlockSpec(memory_space=pl.ANY)] * 8,
        out_specs=[pl.BlockSpec(memory_space=pl.ANY)] * 8,
        out_shape=[jax.ShapeDtypeStruct(a.shape, BF16) for a in outs],
        scratch_shapes=scratch,
        compiler_params=pltpu.CompilerParams(vmem_limit_bytes=126 * 1024 * 1024),
    )(*args)
    out, dx, dw1, dw2, dg, dwf, dwg, dwo = res
    return (out.reshape(grad_out.shape), dx.reshape(x.shape), dw1, dw2,
            dg.reshape(g.shape), dwf, dwg, dwo)
```
